```python
import os as _os
_os.environ.setdefault("JAX_PLATFORMS", "cpu")
import jax
import jax.numpy as jnp

def _softmax(x, axis=-1):
    return jax.nn.softmax(x, axis=axis)
def _gelu(x):
    return jax.nn.gelu(x, approximate=True)
def _silu(x):
    return jax.nn.silu(x)
def _sigmoid(x):
    return jax.nn.sigmoid(x)
def _layernorm(x, axis=-1, eps=1e-5):
    m = jnp.mean(x, axis=axis, keepdims=True)
    v = jnp.var(x, axis=axis, keepdims=True)
    return (x - m) / jnp.sqrt(v + eps)
def _scatter_add(tgt, idx, src, axis=0):
    return tgt.at[idx].add(src)
def _segment_sum(src, seg, n):
    return jax.ops.segment_sum(src, seg, n)
class _Rng:
    def __init__(self, key):
        self._k = key
    def _next(self):
        self._k, sub = jax.random.split(self._k)
        return sub
    def normal(self, shape):
        return jax.random.normal(self._next(), shape, dtype=jnp.bfloat16)
    def randint(self, lo, hi, shape):
        return jax.random.randint(self._next(), shape, lo, hi, dtype=jnp.int32)
    def uniform(self, shape, lo=0.0, hi=1.0):
        return jax.random.uniform(self._next(), shape, jnp.bfloat16, lo, hi)
    def permutation(self, n):
        return jax.random.permutation(self._next(), n)


kernel_name = 'sequential_preLN__sliding_block__swiglu_ffn__prompt'

def setup_inputs():
    _rng = _Rng(jax.random.key(int.from_bytes(__import__("os").urandom(4), "little")))
    _w = (lambda a: (lambda t: t.astype(jnp.bfloat16) if jnp.issubdtype(t.dtype, jnp.floating) else t)(jnp.asarray(a)))
    def _A_setup():
        B, S, D = 1, 2048, 512
        return {
            "x": _w((lambda *s: _rng.normal(s) * 0.05)(B, S, D)),
            "wqkv": _w((lambda *s: _rng.normal(s) * 0.05)(D, 3 * D)),
            "wo": _w((lambda *s: _rng.normal(s) * 0.05)(D, D)),
        }
    _A_in = _A_setup()

    def _B_setup():
        B, S, D, F = 1, 2048, 512, 1792
        return {
            "x": _w((lambda *s: _rng.normal(s) * 0.05)(B, S, D)),
            "w_gate": _w((lambda *s: _rng.normal(s) * 0.05)(D, F)),
            "w_up": _w((lambda *s: _rng.normal(s) * 0.05)(D, F)),
            "w_down": _w((lambda *s: _rng.normal(s) * 0.05)(F, D)),
        }
    _B_in = _B_setup()

    return {
        "A_x": _A_in["x"],
        "A_wqkv": _A_in["wqkv"],
        "A_wo": _A_in["wo"],
        "B_x": _B_in["x"],
        "B_w_gate": _B_in["w_gate"],
        "B_w_up": _B_in["w_up"],
        "B_w_down": _B_in["w_down"],
    }

def reference(A_x, A_wqkv, A_wo, B_x, B_w_gate, B_w_up, B_w_down):
    def _A_ref(x, wqkv, wo):
        B, S, D = x.shape
        H = 32; Dh = D // H; W = 256
        qkv = (lambda x, *d: x.transpose(*d))((x @ wqkv).reshape(B, S, 3, H, Dh), 2, 0, 3, 1, 4)
        q, k, v = qkv[0], qkv[1], qkv[2]
        scores = jnp.einsum("bhqd,bhkd->bhqk", q, k) * (Dh ** -0.5)
        idx = jnp.arange(S)
        mask = (idx[:, None] - idx[None, :] >= 0) & (idx[:, None] - idx[None, :] < W)
        scores = jnp.where(mask[None, None], scores, -1e9)
        p = _softmax(scores, axis=-1)
        o = jnp.einsum("bhqk,bhkd->bhqd", p, v)
        return (lambda x, *d: x.transpose(*d))(o, 0, 2, 1, 3).reshape(B, S, D) @ wo

    def _B_ref(x, w_gate, w_up, w_down):
        g = _silu(x @ w_gate)
        u = x @ w_up
        return (g * u) @ w_down

    x = A_x
    h = x + _A_ref(_layernorm(x, axis=-1), A_wqkv, A_wo)
    h2 = h + _B_ref(_layernorm(h, axis=-1), B_w_gate, B_w_up, B_w_down)
    return h2
```

```python
import functools
import numpy as np
import jax
import jax.numpy as jnp
from jax import lax
import jax.experimental.pallas as pl
import jax.experimental.pallas.tpu as pltpu

S, D, H, DH, WIN, F = 2048, 512, 32, 16, 256, 1792
QB = 128
NG = D // 128
F32, BF16, U32 = jnp.float32, jnp.bfloat16, jnp.uint32
QSCALE = float(DH ** -0.5 * np.log2(np.e))


def _pk(x):
    return pltpu.bitcast(x, U32)


def _upk(x):
    return pltpu.bitcast(x, BF16)


def _dot(a, b):
    return jnp.dot(a, b, preferred_element_type=F32)


def _ln(x):
    m = jnp.mean(x, axis=-1, keepdims=True)
    c = x - m
    v = jnp.mean(c * c, axis=-1, keepdims=True)
    return c * lax.rsqrt(v + 1e-5)


def make(BM=256, FC=256, LOOK=1, NSLOT=2, PM=0, flags=None, parts="qaf"):
    NB = S // BM
    NQ = BM // QB

    def kernel(x_hbm, wqkv_hbm, wo_hbm, wg_hbm, wu_hbm, wd_hbm, out_hbm,
               x_v, wqkv_v, wo_v, wg_v, wu_v, wd_v, out_v,
               k_s, vT_s, qT_s, oT_s, s_s, h_s, hn_s, act_s, in_sem, out_sem):
        def x_copy(b):
            return pltpu.make_async_copy(x_hbm.at[pl.ds(b * BM, BM)], x_v.at[pl.ds(b * BM, BM)], in_sem.at[b])
        w_copies = [pltpu.make_async_copy(s, d, in_sem.at[NB + i]) for i, (s, d) in enumerate(
            [(wqkv_hbm, wqkv_v), (wo_hbm, wo_v), (wg_hbm, wg_v), (wu_hbm, wu_v), (wd_hbm, wd_v)])]
        x_copy(0).start()
        w_copies[0].start()

        t_i = lax.broadcasted_iota(jnp.int32, (64, QB), 0)
        q_i = lax.broadcasted_iota(jnp.int32, (64, QB), 1)
        sel0 = t_i <= q_i
        sel1 = (t_i + 64 <= q_i) | (q_i < 64)
        lo_ok = jnp.where(2 * t_i <= q_i, np.uint32(0x0000FFFF), np.uint32(0))
        hi_ok = jnp.where(2 * t_i + 1 <= q_i, np.uint32(0xFFFF0000), np.uint32(0))
        new_bits = lo_ok | hi_ok
        lane8 = lax.broadcasted_iota(jnp.int32, (8, QB), 1)
        lane64 = q_i < 64
        tri = lax.broadcasted_iota(jnp.int32, (QB, QB), 0) <= lax.broadcasted_iota(jnp.int32, (QB, QB), 1)

        def qkv(b):
            r0 = pl.multiple_of(b * BM, BM)
            xn = _ln(x_v[pl.ds(r0, BM), :].astype(F32)).astype(BF16)
            q = _dot(xn, wqkv_v[:, 0:D]) * QSCALE
            qT_s[...] = _pk(q.T.astype(BF16))
            k = _dot(xn, wqkv_v[:, D:2 * D])
            k_s[pl.ds(pl.multiple_of(b * (BM // 2), BM // 2), BM // 2), :] = _pk(k.astype(BF16))
            v = _dot(xn, wqkv_v[:, 2 * D:3 * D])
            vT = _pk(v.T.astype(BF16))
            for j in range(NQ):
                vT_s[b * NQ + j] = vT[:, j * QB:(j + 1) * QB]

        def krows(j, off, n, g):
            st = j * (QB // 2) + off // 2
            if not isinstance(st, int):
                st = pl.multiple_of(st, 32)
            return k_s[pl.ds(st, n // 2), g * 128:(g + 1) * 128]

        def stationary(pieces):
            z = jnp.zeros((8, QB), U32)
            return _upk(jnp.concatenate([pieces.get(i, z) for i in range(8)], axis=0))

        def scores(j, jl, hq, nt, cache, slot):
            g, half = divmod(hq, 2)
            qs = [qT_s[h * 8:(h + 1) * 8, jl * QB:(jl + 1) * QB] for h in range(4 * hq, 4 * hq + 4)]
            w0 = jnp.concatenate([stationary({4 * half + i: qs[i]}) for i in range(4)], axis=1)
            if nt == 3:
                if (jl, g) not in cache:
                    ko1 = krows(j, -192, 64, g)
                    a = jnp.concatenate([krows(j, 64, 64, g), ko1], axis=0)
                    r = pltpu.roll(jnp.concatenate([ko1, krows(j, -256, 64, g)], axis=0), 64, 1)
                    cache[(jl, g)] = (jnp.where(lane64, a, r), jnp.where(lane64, r, a))
                w1 = jnp.concatenate([stationary({
                    4 * half + i: jnp.where(lane8 >= 64, qs[i], np.uint32(0)),
                    4 * (1 - half) + i: jnp.where(lane8 < 64, qs[i], np.uint32(0))}) for i in range(4)], axis=1)
                sb = _dot(_upk(cache[(jl, g)][half]), w1)
                sa = _dot(_upk(krows(j, -128, 192, g)), w0)
            else:
                sa = _dot(_upk(krows(j, -128 * (nt - 1), 128 * nt, g)), w0)
            ms = []
            for i in range(4):
                c = slice(i * QB, (i + 1) * QB)
                if nt == 3:
                    y = sb[64:, c]
                    parts_ = [sa[:128, c], jnp.where(sel0, sa[128:, c], y), jnp.where(sel1, sb[:64, c], y)]
                else:
                    o = 128 * (nt - 1)
                    parts_ = [sa[:o, c]] * (nt - 1) + [jnp.where(sel0, sa[o:o + 64, c], -1e30),
                                                        jnp.where(t_i + 64 <= q_i, sa[o + 64:, c], -1e30)]
                s = jnp.concatenate(parts_, axis=0)
                s_s[slot, i, :s.shape[0], :] = s
                ms.append(jnp.max(s, axis=0, keepdims=True))
            return ms

        def finish(j, jl, hq, nt, slot, ms):
            for i in range(4):
                h = 4 * hq + i
                p = jnp.exp2(s_s[slot, i, :128 * min(nt, 2), :] - ms[i])
                l = jnp.sum(p, axis=0, keepdims=True)
                if nt == 3:
                    pm = p[128:]
                    if PM == 0:
                        pb = jnp.concatenate([jnp.where(tri, 0.0, pm), p[:128], jnp.where(tri, pm, 0.0)], axis=0).astype(BF16)
                    elif PM == 1:
                        pmb = pm.astype(BF16)
                        z = jnp.zeros_like(pmb)
                        pb = jnp.concatenate([jnp.where(tri, z, pmb), p[:128].astype(BF16), jnp.where(tri, pmb, z)], axis=0)
                    else:
                        pmb = pltpu.pack_elementwise([pm[:64], pm[64:]], packed_dtype=BF16)
                        pn = pmb & new_bits
                        p0 = pltpu.pack_elementwise([p[:64], p[64:128]], packed_dtype=BF16)
                        pb = _upk(jnp.concatenate([pmb ^ pn, p0, pn], axis=0))
                else:
                    pb = p.astype(BF16)
                vh = jnp.concatenate([vT_s[j - (nt - 1) + t, h * 8:(h + 1) * 8, :] for t in range(nt)], axis=1)
                o = _dot(_upk(vh), pb)
                oT_s[h * DH:(h + 1) * DH, jl * QB:(jl + 1) * QB] = o * (1.0 / l)

        def attn(b, first):
            units = [(jl, hq) for jl in range(NQ) for hq in range(H // 4)]
            cache, pend = {}, []
            for u in range(len(units) + LOOK):
                if u < len(units):
                    jl, hq = units[u]
                    nt = min(jl + 1, 3) if first else 3
                    j = jl if first else b * NQ + jl
                    slot = u % NSLOT
                    pend.append((j, jl, hq, nt, slot, scores(j, jl, hq, nt, cache, slot)))
                if u >= LOOK:
                    finish(*pend.pop(0))

        def proj(b):
            r0 = pl.multiple_of(b * BM, BM)
            o = oT_s[...].T.astype(BF16)
            h = x_v[pl.ds(r0, BM), :].astype(F32) + _dot(o, wo_v[...])
            h_s[...] = h
            hn_s[...] = _pk(_ln(h).astype(BF16))

        def ffn(b):
            r0 = pl.multiple_of(b * BM, BM)
            hn = _upk(hn_s[...])
            for c in range(F // FC):
                hg = 0.5 * _dot(hn, wg_v[:, c * FC:(c + 1) * FC])
                u = _dot(hn, wu_v[:, c * FC:(c + 1) * FC])
                act_s[:, c * FC:(c + 1) * FC] = _pk(((hg + hg * jnp.tanh(hg)) * u).astype(BF16))
            y = h_s[...] + _dot(_upk(act_s[...]), wd_v[...])
            out_v[pl.ds(r0, BM), :] = y.astype(BF16)
            pltpu.make_async_copy(out_v.at[pl.ds(r0, BM)], out_hbm.at[pl.ds(r0, BM)], out_sem.at[b]).start()

        x_copy(0).wait()
        w_copies[0].wait()
        for c in w_copies[1:]:
            c.start()
        for b in range(1, NB):
            x_copy(b).start()
        qkv(0)
        attn(0, True)
        w_copies[1].wait()
        proj(0)
        for c in w_copies[2:]:
            c.wait()
        ffn(0)

        def body(b, carry):
            x_copy(b).wait()
            if "q" in parts: qkv(b)
            if "a" in parts: attn(b, False)
            if "q" in parts: proj(b)
            if "f" in parts: ffn(b)
            else:
                r0 = pl.multiple_of(b * BM, BM)
                pltpu.make_async_copy(out_v.at[pl.ds(r0, BM)], out_hbm.at[pl.ds(r0, BM)], out_sem.at[b]).start()
            return carry
        lax.fori_loop(1, NB, body, 0)
        for b in range(NB):
            pltpu.make_async_copy(out_v.at[pl.ds(b * BM, BM)], out_hbm.at[pl.ds(b * BM, BM)], out_sem.at[b]).wait()

    @jax.jit
    def run(A_x, A_wqkv, A_wo, B_x, B_w_gate, B_w_up, B_w_down):
        any_spec = pl.BlockSpec(memory_space=pl.ANY)
        out = pl.pallas_call(
            kernel,
            out_shape=jax.ShapeDtypeStruct((S, D), BF16),
            in_specs=[any_spec] * 6,
            out_specs=any_spec,
            scratch_shapes=[
                pltpu.VMEM((S, D), BF16), pltpu.VMEM((D, 3 * D), BF16), pltpu.VMEM((D, D), BF16),
                pltpu.VMEM((D, F), BF16), pltpu.VMEM((D, F), BF16), pltpu.VMEM((F, D), BF16),
                pltpu.VMEM((S, D), BF16),
                pltpu.VMEM((S // 2, D), U32), pltpu.VMEM((S // QB, D // 2, QB), U32),
                pltpu.VMEM((D // 2, BM), U32), pltpu.VMEM((D, BM), F32), pltpu.VMEM((NSLOT, 4, 256, QB), F32),
                pltpu.VMEM((BM, D), F32), pltpu.VMEM((BM // 2, D), U32), pltpu.VMEM((BM // 2, F), U32),
                pltpu.SemaphoreType.DMA((NB + 5,)), pltpu.SemaphoreType.DMA((NB,)),
            ],
            compiler_params=pltpu.CompilerParams(vmem_limit_bytes=100 * 1024 * 1024, flags=flags),
            name="fused_block",
        )(A_x.reshape(S, D), A_wqkv, A_wo, B_w_gate, B_w_up, B_w_down)
        return out.reshape(1, S, D)
    return run


_run = make()


@jax.jit
def pallas_sequential_preLN__sliding_block__swiglu_ffn__prompt_kernel(A_x, A_wqkv, A_wo, B_x, B_w_gate, B_w_up, B_w_down):
    return _run(A_x, A_wqkv, A_wo, B_x, B_w_gate, B_w_up, B_w_down)
```

```python
import contextlib
import numpy as np
import jax
import jax.numpy as jnp
from jax import lax
import jax.experimental.pallas as pl
import jax.experimental.pallas.tpu as pltpu

S, D, H, DH, F = 2048, 512, 32, 16, 1792
QB = 128
F32, BF16, U32 = jnp.float32, jnp.bfloat16, jnp.uint32
QSCALE = float(DH ** -0.5 * np.log2(np.e))
NEG = -1e30


def _pk(x):
    return pltpu.bitcast(x, U32)


def _upk(x):
    return pltpu.bitcast(x, BF16)


def _dot(a, b):
    return jnp.dot(a, b, preferred_element_type=F32)


def _ln(x, scale=1.0):
    m = jnp.mean(x, axis=-1, keepdims=True)
    c = x - m
    v = jnp.mean(c * c, axis=-1, keepdims=True)
    r = lax.rsqrt(v + 1e-5)
    return c * (r if scale == 1.0 else r * scale)


def _lhs7(a11, a12, a21, a22):
    return [a11 + a22, a21 + a22, a11, a22, a11 + a12, a21 - a11, a12 - a22]


def _rhs5(b11, b12, b21, b22):
    return [b11 + b22, b12 - b22, b21 - b11, b11 + b12, b21 + b22]


def _strassen(prod):
    m5 = prod(4)
    yield
    m3 = prod(2)
    c12 = m5 + m3
    yield
    m1 = prod(0)
    c11, c22 = m1 - m5, m1 + m3
    yield
    c11 = c11 + prod(6)
    yield
    m4 = prod(3)
    c11 = c11 + m4
    yield
    m2 = prod(1)
    c21, c22 = m4 + m2, c22 - m2
    yield
    c22 = c22 + prod(5)
    return c11, c12, c21, c22


RHS_SLOT = (0, None, 1, 2, None, 3, 4)


def _mix(*streams):
    toks = []
    for s_ in streams:
        t = s_.split()
        if not t:
            continue
        toks += [((i + 0.5) / len(t), len(toks) + i, x) for i, x in enumerate(t)]
    return " ".join(x for _, _, x in sorted(toks)) + " "


def _t(kind, b, n=1):
    return f"{kind}{b} " * n


def make(NSL=8, LOOK=1, LNS=64, PH=0, GZ=0, Q1=21, R0=32, NWD=2, V0=0, V1=0, V2=0, VL=2, flags=None, PROF=0):
    BM = 256
    NB = S // BM
    NQ = BM // QB
    HM, HD, HF, HQ = BM // 2, D // 2, F // 2, 3 * D // 2
    HPT = 8 // NSL
    SW = QB // NSL
    NU = NQ * (H // 4)
    NCH = HF // 128
    NSLOT = LOOK + 1
    NL = HM // LNS * (3 if PH else 1)
    UNITS = [(jl, hq) for part in ((0, 1, 4, 5), (2, 3, 6, 7)) for jl in range(NQ) for hq in part]

    def att(b):
        o = _t("s", b, LOOK)
        for u in range(NU):
            o += (_t("s", b) if u + LOOK < NU else "") + _t("f", b, 4) + (_t("o", b) if u + 1 in (NU // 2, NU) else "")
        return o

    def attend(a, side=""):
        return _mix(att(a), _t("g", a - 1, 98) + _t("z", 0, GZ), side)

    def project(a, with_q=True):
        f, q = a - 1, a + 1
        if not with_q:
            return _t("D", f, 3) + _t("p", a, 14) + _t("D", f) + _mix(_t("D", f, 2), _t("l", a, NL)) + _t("D", f) + _t("c", f)
        o = _mix(_t("D", f, 3), _t("n", q, NL) + _t("z", 0, 1))
        if VL == 0:
            return o + _t("p", a, 14) + _t("q", q, 7) + _mix(_t("q", q, 35), _t("l", a, NL), _t("D", f, 2)) + _t("D", f, 2) + _t("c", f)
        if VL == 1:
            return o + _t("p", a, 14) + _t("q", q, 7) + _mix(_t("q", q, 21), _t("l", a, NL)) + _t("q", q, 14) + _t("D", f, 4) + _t("c", f)
        if VL == 2:
            return o + _t("q", q, 14) + _t("p", a, 14) + _t("q", q, 7) + _mix(_t("q", q, 21), _t("l", a, NL), _t("D", f, 2)) + _t("D", f, 2) + _t("c", f)
        if VL == 3:
            return o + _t("q", q, 42) + _t("p", a, 14) + _t("D", f) + _mix(_t("D", f, 2), _t("l", a, NL)) + _t("D", f) + _t("c", f)
    head = "Wx0 n0 Wq B " + _t("q", 0, 4) + "Wk " + _t("q", 0, 4) + "Wv Wx1 Wo " + _mix(_t("q", 0, 4), _t("t", 0, 24))
    head += _mix(att(0), _t("n", 1, NL) + _t("q", 1, Q1) + _t("z", 0, 2), _t("t", 0, 72) + _t("u", 0, 32) + _t("z", 0, V0))
    rest = 42 - Q1
    head += _t("q", 1, rest // 3) + _t("p", 0, 14) + _t("q", 1, rest // 3) + "Wg X "
    head += _mix(_t("q", 1, rest - 2 * (rest // 3)), _t("l", 0, NL), _t("r", 0, R0))
    if V1 == 0:
        head += attend(1, _t("r", 0, 224 - R0) + "Wd " + _t("r", 0, 112)) + "Wx2 "
    else:
        head += "Wd " + attend(1, _t("r", 0, 336 - R0)) + "Wx2 "
    tail = project(NB - 1, False) + _t("g", NB - 1, 98) + _t("D", NB - 1, 6) + "C1 " + _t("D", NB - 1) + "C0"

    def kernel(x_hbm, wqkv_hbm, wo_hbm, wg_hbm, wu_hbm, wd_hbm, out_hbm,
               x_v, wqkv_v, wo_v, wg_v, wu_v, wd_v, out_v, rq_s, ro_s, rg_s, rd_s,
               lx_s, lo_s, l1_s, l2_s, k_s, vT_s, qT_s, oT_s, s_s, h_s, y_s, in_sem, out_sem):
        rq_s, ro_s, rg_s, rd_s, lx_s, lo_s, l1_s, l2_s = (
            r.bitcast(BF16) for r in (rq_s, ro_s, rg_s, rd_s, lx_s, lo_s, l1_s, l2_s))

        def al(i, n):
            return i if isinstance(i, int) else pl.multiple_of(i, n)

        def x_copy(b0, nb, i):
            return pltpu.make_async_copy(x_hbm.at[pl.ds(b0 * BM, nb * BM)], x_v.at[pl.ds(b0 * BM, nb * BM)], in_sem.at[i])

        def out_copy(b):
            r = pl.ds(al(b * BM, BM), BM)
            return pltpu.make_async_copy(out_v.at[r], out_hbm.at[r], out_sem.at[b])

        def half_copy(i):
            r = pl.ds((NB - 1) * BM + i * HM, HM)
            return pltpu.make_async_copy(out_v.at[r], out_hbm.at[r], out_sem.at[NB - 1 + i])
        x_copies = [x_copy(0, 1, 0), x_copy(1, 2, 1), x_copy(3, NB - 3, 2)]
        sem_ids = iter(range(3, 64))

        def split_copy(src, dst, n):
            rows = src.shape[0] // n
            return [pltpu.make_async_copy(src.at[pl.ds(i * rows, rows)], dst.at[pl.ds(i * rows, rows)],
                                          in_sem.at[next(sem_ids)]) for i in range(n)]
        qkv_copies = [pltpu.make_async_copy(wqkv_hbm.at[:, pl.ds(i * D, D)], wqkv_v.at[:, pl.ds(i * D, D)],
                                            in_sem.at[next(sem_ids)]) for i in range(3)]
        w_copies = [split_copy(wo_hbm, wo_v, 1), split_copy(wg_hbm, wg_v, NWD) + split_copy(wu_hbm, wu_v, NWD),
                    split_copy(wd_hbm, wd_v, NWD)]
        x_copies[0].start()
        for c in qkv_copies:
            c.start()

        lane = lax.broadcasted_iota(jnp.int32, (8, QB), 1)
        tri = lax.broadcasted_iota(jnp.int32, (QB, QB), 0) <= lax.broadcasted_iota(jnp.int32, (QB, QB), 1)

        def store_lhs7(dst, a11, a12, a21, a22, cs=slice(None), r0=0):
            for i, a in enumerate(_lhs7(a11, a12, a21, a22)):
                dst[i * HM + r0:i * HM + r0 + a.shape[0], cs] = a.astype(BF16)

        def prep_rhs(dst, kh, quad, tiles):
            for r0, c0 in tiles:
                r = _rhs5(*(ref[ro + r0:ro + r0 + 16, co + c0:co + c0 + 128].astype(F32) for ref, ro, co in quad))
                for i in range(5):
                    dst[i * kh + r0:i * kh + r0 + 16, c0:c0 + 128] = r[i].astype(BF16)
                yield

        def rhs(i, pre, kh, quad, cs):
            if RHS_SLOT[i] is None:
                ref, ro, co = quad[0 if i == 1 else 3]
                return ref[ro:ro + kh, co + cs.start:co + cs.stop]
            return pre[RHS_SLOT[i] * kh:(RHS_SLOT[i] + 1) * kh, cs]
        quad_q = ((wqkv_v, 0, 0), (wqkv_v, 0, HQ), (wqkv_v, HD, 0), (wqkv_v, HD, HQ))
        quad_o = ((wo_v, 0, 0), (wo_v, 0, HD), (wo_v, HD, 0), (wo_v, HD, HD))
        quad_g = ((wg_v, 0, 0), (wu_v, 0, 0), (wg_v, HD, 0), (wu_v, HD, 0))
        quad_d = ((wd_v, 0, 0), (wd_v, 0, HD), (wd_v, HF, 0), (wd_v, HF, HD))

        def ln_steps(load, dst, scale):
            slabs = range(0, HM, LNS)
            mean, rstd = {}, {}
            for r in slabs:
                for o in (r, HM + r):
                    mean[o] = jnp.mean(load(o), axis=-1, keepdims=True)
                if PH:
                    yield
            for r in slabs:
                for o in (r, HM + r):
                    c = load(o) - mean[o]
                    rstd[o] = lax.rsqrt(jnp.mean(c * c, axis=-1, keepdims=True) + 1e-5) * scale
                if PH:
                    yield
            for r in slabs:
                top, bot = ((load(o) - mean[o]) * rstd[o] for o in (r, HM + r))
                store_lhs7(dst, top[:, :HD], top[:, HD:], bot[:, :HD], bot[:, HD:], r0=r)
                yield

        def ln1_steps(b, plain):
            if plain:
                xn = _ln(x_v[b * BM:(b + 1) * BM, :].astype(F32))
                lx_s[0:BM, :], lx_s[BM:2 * BM, :] = xn[:, :HD].astype(BF16), xn[:, HD:].astype(BF16)
                yield
            else:
                yield from ln_steps(lambda o: x_v[pl.ds(al(b * BM + o, LNS), LNS), :].astype(F32), lx_s, 1.0)

        def put_qkv(b, jl, ct, val):
            kind, g = divmod(ct, D // 128)
            j = b * NQ + jl
            if kind == 0:
                qT_s[pl.ds(al(j * HD + g * 64, 64), 64), :] = _pk((val * QSCALE).T.astype(BF16))
            elif kind == 2:
                vT_s[pl.ds(al(j * HD + g * 64, 64), 64), :] = _pk(val.T.astype(BF16))
            else:
                ln_ = lax.broadcasted_iota(jnp.int32, (QB // 2, 128), 1)
                tiles, w = [_pk(val.astype(BF16))], 64
                while w >= SW:
                    first = (ln_ & w) == 0
                    nxt = []
                    for t in tiles:
                        r = pltpu.roll(t, w, 1)
                        nxt += [jnp.where(first, t, r), jnp.where(first, r, t)]
                    tiles, w = nxt, w // 2
                for i, t in enumerate(tiles):
                    k_s[g * NSL + i, pl.ds(al(j * (QB // 2), QB // 2), QB // 2), :] = t

        def qkv_steps(b, plain):
            if plain:
                for ct in range(3 * D // 128):
                    cs = slice(ct * 128, (ct + 1) * 128)
                    val = _dot(jnp.concatenate([lx_s[0:BM, :], lx_s[BM:2 * BM, :]], axis=1), wqkv_v[:, cs])
                    for jl in range(NQ):
                        put_qkv(b, jl, ct, val[jl * QB:(jl + 1) * QB])
                    yield
                return
            for ct in range(HQ // 128):
                cs = slice(ct * 128, (ct + 1) * 128)
                c11, c12, c21, c22 = yield from _strassen(
                    lambda i: _dot(lx_s[i * HM:(i + 1) * HM, :], rhs(i, rq_s, HD, quad_q, cs)))
                for jl, c_, val in ((0, ct, c11), (0, ct + HQ // 128, c12), (1, ct, c21), (1, ct + HQ // 128, c22)):
                    put_qkv(b, jl, c_, val)
                yield

        def krows(t, j, off, n):
            return k_s[t, pl.ds(al(j * (QB // 2) + off // 2, 8), n // 2), :]

        def scores(j, jl, hq, nt, slot):
            ms = []
            for t in range(4 * hq // HPT, (4 * hq + 4) // HPT):
                z = jnp.zeros((8, QB), U32)
                ws = []
                for e in range(HPT):
                    h = t * HPT + e
                    qh = qT_s[pl.ds(al(j * (D // 2) + h * 8, 8), 8), :]
                    if nt == 3:
                        pcs = [jnp.where((lane >= (i // HPT) * SW) & (lane < (i // HPT + 1) * SW), qh, np.uint32(0))
                               if i % HPT == e else z for i in range(8)]
                    else:
                        pcs = [qh if i == e else z for i in range(8)]
                    ws.append(jnp.concatenate(pcs, axis=0))
                w = _upk(jnp.concatenate(ws, axis=1))
                if nt == 3:
                    lhs = [krows(t, j, -128, 128 + SW)]
                    ln_ = lax.broadcasted_iota(jnp.int32, (SW // 2, 128), 1)
                    edge = None
                    for c in range(NSL):
                        old = krows(t, j, -256 + c * SW, SW)
                        edge = old if c == 0 else jnp.where(ln_ >= c * SW, old, edge)
                        if c > 0:
                            lhs.append(jnp.where(ln_ >= c * SW, krows(t, j, c * SW, SW), old))
                    s_all = _dot(_upk(jnp.concatenate([edge] + lhs, axis=0)), w)
                else:
                    s_all = _dot(_upk(krows(t, j, -128 * (nt - 1), 128 * nt)), w)
                for e in range(HPT):
                    s = s_all[:, e * QB:(e + 1) * QB]
                    if nt == 3:
                        r_ = lax.broadcasted_iota(jnp.int32, (SW, QB), 0)
                        c_ = lax.broadcasted_iota(jnp.int32, (SW, QB), 1)
                        parts = [s[SW:SW + 128]]
                        for c in range(NSL):
                            use_old = (c_ >= c * SW) & (c_ < c * SW + r_)
                            parts.append(jnp.where(use_old, s[:SW], s[SW + 128 + c * SW:2 * SW + 128 + c * SW]))
                    else:
                        o = 128 * (nt - 1)
                        parts = [s[:o]] * (nt - 1) + [jnp.where(tri, s[o:], NEG)]
                    s = jnp.concatenate(parts, axis=0)
                    s_s[slot, len(ms), :s.shape[0], :] = s
                    ms.append(jnp.max(s, axis=0, keepdims=True))
            return ms

        def finish_steps(pend):
            while True:
                j, jl, hq, nt, slot, ms = pend.pop(0)
                for i in range(4):
                    h = 4 * hq + i
                    p = jnp.exp2(s_s[slot, i, :128 * min(nt, 2), :] - ms[i])
                    l = jnp.sum(p, axis=0, keepdims=True)
                    if nt == 3:
                        p = jnp.concatenate([jnp.where(tri, 0.0, p[128:]), p[:128], jnp.where(tri, p[128:], 0.0)], axis=0)
                    vh = jnp.concatenate([vT_s[pl.ds(al((j - (nt - 1) + t) * (D // 2) + h * 8, 8), 8), :]
                                          for t in range(nt)], axis=1)
                    o = _dot(_upk(vh), p.astype(BF16))
                    oT_s[h * DH:(h + 1) * DH, jl * QB:(jl + 1) * QB] = o * (1.0 / l)
                    yield

        def score_steps(b, first, pend):
            for u, (jl, hq) in enumerate(UNITS):
                nt = min(jl + 1, 3) if first else 3
                j = b * NQ + jl
                pend.append((j, jl, hq, nt, u % NSLOT, scores(j, jl, hq, nt, u % NSLOT)))
                yield

        def prep_o_steps():
            for c in range(0, HD, 128):
                store_lhs7(lo_s, *(oT_s[f0 + c:f0 + c + 128, t0:t0 + HM].T for t0 in (0, HM) for f0 in (0, HD)),
                           cs=slice(c, c + 128))
                yield

        def proj_steps(b):
            for ct in range(HD // 128):
                cs = slice(ct * 128, (ct + 1) * 128)
                c = yield from _strassen(lambda i: _dot(lo_s[i * HM:(i + 1) * HM, :], rhs(i, ro_s, HD, quad_o, cs)))
                for k in range(4):
                    r0, c0 = k // 2 * HM, k % 2 * HD + ct * 128
                    h_s[r0:r0 + HM, c0:c0 + 128] = x_v[pl.ds(al(b * BM + r0, HM), HM), c0:c0 + 128].astype(F32) + c[k]
                yield

        def ln2_steps():
            return ln_steps(lambda o: h_s[o:o + LNS, :], l1_s, 0.5)

        def act(hg, hu):
            return (hg + hg * jnp.tanh(hg)) * hu

        def gate_up_steps():
            for c in range(NCH):
                quad = []
                for cs in (slice(c * 128, (c + 1) * 128), slice(HF + c * 128, HF + (c + 1) * 128)):
                    g_t, u_t, g_b, u_b = yield from _strassen(
                        lambda i: _dot(l1_s[i * HM:(i + 1) * HM, :], rhs(i, rg_s, HD, quad_g, cs)))
                    quad.append((act(g_t, u_t), act(g_b, u_b)))
                    if len(quad) == 2:
                        store_lhs7(l2_s, quad[0][0], quad[1][0], quad[0][1], quad[1][1], slice(c * 128, (c + 1) * 128))
                    yield

        T, Bo, Lf, Rt = slice(0, HM), slice(HM, BM), slice(0, HD), slice(HD, D)
        DOWN = [[((T, Lf), 1), ((Bo, Rt), 1)], [((Bo, Lf), 1), ((Bo, Rt), -1)], [((T, Rt), 1), ((Bo, Rt), 1)],
                [((T, Lf), 1), ((Bo, Lf), 1)], [((T, Lf), -1), ((T, Rt), 1)], [((Bo, Rt), 1)], [((T, Lf), 1)]]

        def down_steps(b):
            for i in range(7):
                m = _dot(l2_s[i * HM:(i + 1) * HM, :], rhs(i, rd_s, HF, quad_d, slice(0, HD)))
                for (rs, cs), sg in DOWN[i]:
                    seen = [k for k in range(7) if any(q == (rs, cs) for q, _ in DOWN[k])]
                    acc = 0.5 * h_s[rs, cs] if i == seen[0] else y_s[rs, cs]
                    acc = acc + m if sg > 0 else acc - m
                    if i == seen[-1]:
                        out_v[pl.ds(al(b * BM + rs.start, HM), HM), cs] = (2.0 * acc).astype(BF16)
                    else:
                        y_s[rs, cs] = acc
                yield

        def start(copies):
            return lambda: [c.start() for c in copies]

        def wait(copies):
            return lambda: [c.wait() for c in copies]

        def chain(*gens):
            for g in gens:
                yield from g
        prep_q = prep_rhs(rq_s, HD, quad_q, [(r, c) for c in range(0, HQ, 128) for r in range(0, HD, 16)])
        prep_w = prep_rhs(ro_s, HD, quad_o, [(r, c) for c in range(0, HD, 128) for r in range(0, HD, 16)])
        prep_f = chain(
            prep_rhs(rg_s, HD, quad_g, [(r, c + o) for c in range(0, HF, 128) for o in (0, HF) for r in range(0, HD, 16)]),
            prep_rhs(rd_s, HF, quad_d, [(r, c) for r in range(0, HF, 16) for c in range(0, HD, 128)]))

        acts = dict(B=start([x_copies[1]] + sum(w_copies, [])), X=start(x_copies[2:]), Wx0=wait(x_copies[:1]),
                    Wx1=wait(x_copies[1:2]), Wx2=wait(x_copies[2:]), Wq=wait(qkv_copies[:1]), Wk=wait(qkv_copies[1:2]), Wv=wait(qkv_copies[2:]), Wo=wait(w_copies[0]),
                    Wg=wait(w_copies[1]), Wd=wait(w_copies[2]), C0=start([half_copy(0)]), C1=start([half_copy(1)]))

        def run(order, base, tag):
            gens, pend = {}, {}
            with (jax.named_scope(tag) if PROF else contextlib.nullcontext()):
                for it, tok in enumerate(order.split()):
                    if PROF > 1 and it % PROF == 0 and tag == "P0":
                        with jax.named_scope(f"AZ{it}{tok}"):
                            y_s[0:8, 0:128] = y_s[0:8, 0:128] + 0.0
                    if tok in acts:
                        with (jax.named_scope("A" + tok) if PROF else contextlib.nullcontext()):
                            acts[tok]()
                        continue
                    kind, b = tok[0], base + int(tok[1:])
                    if kind == "z":
                        continue
                    if kind == "c":
                        out_copy(b).start()
                        continue
                    if tok not in gens:
                        first = isinstance(b, int) and b == 0
                        q = pend.setdefault(tok[1:], [])
                        gens[tok] = dict(
                            n=lambda: ln1_steps(b, first), q=lambda: qkv_steps(b, first), s=lambda: score_steps(b, first, q),
                            f=lambda: finish_steps(q), o=prep_o_steps, p=lambda: proj_steps(b), l=ln2_steps,
                            g=gate_up_steps, D=lambda: down_steps(b), t=lambda: prep_q, u=lambda: prep_w,
                            r=lambda: prep_f)[kind]()
                    next(gens[tok])

        run(head, 0, "P0")

        def body(b, carry):
            run(project(0) + attend(1), b, "P3")
            return carry
        lax.fori_loop(1, NB - 1, body, 0)
        run(tail, 0, "P4")
        for c in [out_copy(b) for b in range(NB - 1)] + [half_copy(0), half_copy(1)]:
            c.wait()

    @jax.jit
    def call(A_x, A_wqkv, A_wo, B_x, B_w_gate, B_w_up, B_w_down):
        any_spec = pl.BlockSpec(memory_space=pl.ANY)
        out = pl.pallas_call(
            kernel,
            out_shape=jax.ShapeDtypeStruct((S, D), BF16),
            in_specs=[any_spec] * 6,
            out_specs=any_spec,
            scratch_shapes=[
                pltpu.VMEM((S, D), BF16), pltpu.VMEM((D, 3 * D), BF16), pltpu.VMEM((D, D), BF16),
                pltpu.VMEM((D, F), BF16), pltpu.VMEM((D, F), BF16), pltpu.VMEM((F, D), BF16), pltpu.VMEM((S, D), BF16),
                pltpu.VMEM((5 * HD // 2, HQ), U32), pltpu.VMEM((5 * HD // 2, HD), U32),
                pltpu.VMEM((5 * HD // 2, F), U32), pltpu.VMEM((5 * HF // 2, HD), U32),
                pltpu.VMEM((7 * HM // 2, HD), U32), pltpu.VMEM((7 * HM // 2, HD), U32),
                pltpu.VMEM((7 * HM // 2, HD), U32), pltpu.VMEM((7 * HM // 2, HF), U32),
                pltpu.VMEM((NSL * D // 128, S // 2, 128), U32),
                pltpu.VMEM((S // QB * D // 2, QB), U32), pltpu.VMEM((S // QB * D // 2, QB), U32),
                pltpu.VMEM((D, BM), F32), pltpu.VMEM((NSLOT, 4, 256, QB), F32),
                pltpu.VMEM((BM, D), F32), pltpu.VMEM((BM, D), F32),
                pltpu.SemaphoreType.DMA((7 + 3 * NWD,)), pltpu.SemaphoreType.DMA((NB + 1,)),
            ],
            compiler_params=pltpu.CompilerParams(vmem_limit_bytes=100 * 1024 * 1024, flags=flags),
            name="fused_block",
        )(A_x.reshape(S, D), A_wqkv, A_wo, B_w_gate, B_w_up, B_w_down)
        return out.reshape(1, S, D)
    return call


_run = make()


@jax.jit
def pallas_sequential_preLN__sliding_block__swiglu_ffn__prompt_kernel(A_x, A_wqkv, A_wo, B_x, B_w_gate, B_w_up, B_w_down):
    return _run(A_x, A_wqkv, A_wo, B_x, B_w_gate, B_w_up, B_w_down)
```

```python
import numpy as np
import jax
import jax.numpy as jnp
from jax import lax
import jax.experimental.pallas as pl
import jax.experimental.pallas.tpu as pltpu

S, D, H, DH, F = 2048, 512, 32, 16, 1792
QB = 128
F32, BF16, U32 = jnp.float32, jnp.bfloat16, jnp.uint32
QSCALE = float(DH ** -0.5 * np.log2(np.e))
NEG = -1e30
BM = 256
NB, NQ = S // BM, BM // QB
HM, QM, HD, HF, HQ = BM // 2, BM // 4, D // 2, F // 2, 3 * D // 2
NSL, SW = 8, 16
NU = NQ * (H // 4)
NCH = HF // 128
LN1, LN2, KR = 64, 16, 32
UNITS = [(jl, hq) for part in ((0, 1, 4, 5), (2, 3, 6, 7)) for jl in range(NQ) for hq in part]


def _pk(x):
    return pltpu.bitcast(x, U32)


def _upk(x):
    return pltpu.bitcast(x, BF16)


def _dot(a, b):
    return jnp.dot(a, b, preferred_element_type=F32)


def _ln(x, scale=1.0):
    m = jnp.mean(x, axis=-1, keepdims=True)
    c = x - m
    v = jnp.mean(c * c, axis=-1, keepdims=True)
    r = lax.rsqrt(v + 1e-5)
    return c * (r if scale == 1.0 else r * scale)


def _lhs7(a11, a12, a21, a22):
    return [a11 + a22, a21 + a22, a11, a22, a11 + a12, a21 - a11, a12 - a22]


def _rhs5(b11, b12, b21, b22):
    return [b11 + b22, b12 - b22, b21 - b11, b11 + b12, b21 + b22]


def _rhs7(b11, b12, b21, b22):
    return [b11 + b22, b11, b12 - b22, b21 - b11, b22, b11 + b12, b21 + b22]


def _strassen(prod):
    m5 = prod(4)
    yield
    m3 = prod(2)
    c12 = m5 + m3
    yield
    m1 = prod(0)
    c11, c22 = m1 - m5, m1 + m3
    yield
    c11 = c11 + prod(6)
    yield
    m4 = prod(3)
    c11 = c11 + m4
    yield
    m2 = prod(1)
    c21, c22 = m4 + m2, c22 - m2
    yield
    c22 = c22 + prod(5)
    return c11, c12, c21, c22


RHS_SLOT = (0, None, 1, 2, None, 3, 4)
RHS_TERMS = ((0, 1, 3), (0, 0, 0), (1, -1, 3), (2, -1, 0), (3, 0, 0), (0, 1, 1), (2, 1, 3))


def _mix(*streams):
    toks = []
    for s_ in streams:
        t = s_.split()
        if not t:
            continue
        toks += [((i + 0.5) / len(t), len(toks) + i, x) for i, x in enumerate(t)]
    return " ".join(x for _, _, x in sorted(toks)) + " "


def _t(kind, b, n=1):
    return f"{kind}{b} " * n


def _schedule():
    def att(b):
        o = _t("s", b)
        for u in range(NU):
            o += _t("s", b, int(u + 1 < NU)) + _t("f", b, 4) + _t("o", b, int(u + 1 in (NU // 2, NU)))
        return o.split()

    def qk(b):
        return 2 * _mix(_t("q", b, 14), _t("k", b, 2 * NQ * 64 // KR))
    join = " ".join
    ng, nl2, nk = 49 * NCH, QM // LN2, NQ * 64 // KR
    a0, a1 = att(0), att(1)
    head = "Wx0 n0 Wq B " + _t("q", 0, 4) + "Wk q0 " + _mix(_t("q", 0, 3), _t("k", 0, 2 * nk)) + _t("t", 0, 16)
    head += "Wv Wx1 " + _mix(_t("q", 0, 4), _t("k", 0, 2 * nk), _t("t", 0, 8))
    head += _mix(join(a0[:50]), _t("n", 1, HM // LN1) + _t("z", 0, 4) + _t("q", 1, 14), _t("t", 0, 72) + _t("z", 0, 40))
    head += _mix(join(a0[50:]), qk(1)) + "Wo Wg X " + _mix(join(a1[:31]), _t("u", 0, 32) + _t("r", 0, 20))
    head += _mix(join(a1[31:41]), _t("p", 0, 14)) + _mix(join(a1[41:51]), _t("l", 0, nl2))
    head += _mix(join(a1[51:]), _t("g", 0, ng), _t("r", 0, 36) + _t("z", 0, 5) + "Wd " + _t("d", 0, 28)) + "Wx2"
    body = _mix(_t("D", -1, 3), _t("n", 1, HM // LN1) + "z0") + _t("q", 1, 14) + qk(1) + _t("p", 0, 7)
    body += _mix(_t("p", 0, 7) + _t("z", 0, 7) + _mix(_t("l", 0, nl2), _t("z", 0, 12)), _t("D", -1, 4), join(a1[:16]))
    body += _mix(join(a1[16:]), _t("g", 0, ng)) + _t("c", -1)
    tail = _t("D", -1, 3) + _t("p", 0, 14) + _t("D", -1) + _mix(_t("D", -1, 2), _t("l", 0, nl2)) + _t("D", -1) + _t("c", -1)
    tail += _t("g", 0, ng) + _t("D", 0, 6) + "C1 D0 C0"
    return head, body, tail


def _kernel(x_hbm, wqkv_hbm, wo_hbm, wg_hbm, wu_hbm, wd_hbm, out_hbm,
           x_v, wqkv_v, wo_v, wg_v, wu_v, wd_v, out_v, rq_s, ro_s, rg_s, rd_s,
           lx_s, lo_s, l1_s, l2_s, kt_s, k_s, vT_s, qT_s, oT_s, s_s, h_s, y_s, part_s, in_sem, out_sem):
    rq_s, ro_s, rg_s, rd_s, lx_s, lo_s, l2_s = (
        r.bitcast(BF16) for r in (rq_s, ro_s, rg_s, rd_s, lx_s, lo_s, l2_s))

    def al(i, n):
        return i if isinstance(i, int) else pl.multiple_of(i, n)

    def x_copy(b0, nb, i):
        return pltpu.make_async_copy(x_hbm.at[pl.ds(b0 * BM, nb * BM)], x_v.at[pl.ds(b0 * BM, nb * BM)], in_sem.at[i])

    def out_copy(b):
        r = pl.ds(al(b * BM, BM), BM)
        return pltpu.make_async_copy(out_v.at[r], out_hbm.at[r], out_sem.at[b])

    def half_copy(i):
        r = pl.ds((NB - 1) * BM + i * HM, HM)
        return pltpu.make_async_copy(out_v.at[r], out_hbm.at[r], out_sem.at[NB - 1 + i])
    x_copies = [x_copy(0, 1, 0), x_copy(1, 1, 1), x_copy(2, NB - 2, 2)]
    sem_ids = iter(range(3, 64))

    def split_copy(src, dst, n):
        rows = src.shape[0] // n
        return [pltpu.make_async_copy(src.at[pl.ds(i * rows, rows)], dst.at[pl.ds(i * rows, rows)],
                                      in_sem.at[next(sem_ids)]) for i in range(n)]
    qkv_copies = [pltpu.make_async_copy(wqkv_hbm.at[:, pl.ds(i * D, D)], wqkv_v.at[:, pl.ds(i * D, D)],
                                        in_sem.at[next(sem_ids)]) for i in range(3)]
    w_copies = [split_copy(wo_hbm, wo_v, 1), split_copy(wg_hbm, wg_v, 2) + split_copy(wu_hbm, wu_v, 2),
                split_copy(wd_hbm, wd_v, 2)]
    x_copies[0].start()
    for c in qkv_copies:
        c.start()

    lane = lax.broadcasted_iota(jnp.int32, (8, QB), 1)
    tri = lax.broadcasted_iota(jnp.int32, (QB, QB), 0) <= lax.broadcasted_iota(jnp.int32, (QB, QB), 1)

    def store_lhs7(dst, a11, a12, a21, a22, cs=slice(None), r0=0):
        for i, a in enumerate(_lhs7(a11, a12, a21, a22)):
            dst[i * HM + r0:i * HM + r0 + a.shape[0], cs] = a.astype(BF16)

    def prep_rhs(dst, kh, quad, tiles):
        for r0, c0 in tiles:
            r = _rhs5(*(ref[ro + r0:ro + r0 + 16, co + c0:co + c0 + 128].astype(F32) for ref, ro, co in quad))
            for i in range(5):
                dst[i * kh + r0:i * kh + r0 + 16, c0:c0 + 128] = r[i].astype(BF16)
            yield

    def rhs(i, pre, kh, quad, cs):
        if RHS_SLOT[i] is None:
            ref, ro, co = quad[0 if i == 1 else 3]
            return ref[ro:ro + kh, co + cs.start:co + cs.stop]
        return pre[RHS_SLOT[i] * kh:(RHS_SLOT[i] + 1) * kh, cs]
    quad_q = ((wqkv_v, 0, 0), (wqkv_v, 0, HQ), (wqkv_v, HD, 0), (wqkv_v, HD, HQ))
    quad_o = ((wo_v, 0, 0), (wo_v, 0, HD), (wo_v, HD, 0), (wo_v, HD, HD))
    quad_g = ((wg_v, 0, 0), (wu_v, 0, 0), (wg_v, HD, 0), (wu_v, HD, 0))
    quad_d = ((wd_v, 0, 0), (wd_v, 0, HD), (wd_v, HF, 0), (wd_v, HF, HD))

    def ln1_steps(b, plain):
        if plain:
            xn = _ln(x_v[b * BM:(b + 1) * BM, :].astype(F32))
            lx_s[0:BM, :], lx_s[BM:2 * BM, :] = xn[:, :HD].astype(BF16), xn[:, HD:].astype(BF16)
            yield
        else:
            for r in range(0, HM, LN1):
                top, bot = (_ln(x_v[pl.ds(al(b * BM + o + r, LN1), LN1), :].astype(F32)) for o in (0, HM))
                store_lhs7(lx_s, top[:, :HD], top[:, HD:], bot[:, :HD], bot[:, HD:], r0=r)
                yield

    def put_qkv(b, jl, ct, val):
        kind, g = divmod(ct, D // 128)
        j = b * NQ + jl
        if kind == 0:
            qT_s[pl.ds(al(j * HD + g * 64, 64), 64), :] = _pk((val * QSCALE).T.astype(BF16))
        elif kind == 2:
            vT_s[pl.ds(al(j * HD + g * 64, 64), 64), :] = _pk(val.T.astype(BF16))
        else:
            kt_s[(g * NQ + jl) * 64:(g * NQ + jl + 1) * 64, :] = _pk(val.astype(BF16))

    def key_steps(b, plain):
        ln_ = lax.broadcasted_iota(jnp.int32, (KR, 128), 1)
        for g in (range(D // 128) if plain else (2, 0, 3, 1)):
            for r in range(0, NQ * 64, KR):
                tiles, w = [kt_s[g * NQ * 64 + r:g * NQ * 64 + r + KR, :]], 64
                while w >= SW:
                    first = (ln_ & w) == 0
                    nxt = []
                    for t in tiles:
                        rot = pltpu.roll(t, w, 1)
                        nxt += [jnp.where(first, t, rot), jnp.where(first, rot, t)]
                    tiles, w = nxt, w // 2
                for i, t in enumerate(tiles):
                    k_s[g * NSL + i, pl.ds(al(b * HM + r, KR), KR), :] = t
                yield

    def qkv_steps(b, plain):
        if plain:
            for ct in range(3 * D // 128):
                cs = slice(ct * 128, (ct + 1) * 128)
                val = _dot(jnp.concatenate([lx_s[0:BM, :], lx_s[BM:2 * BM, :]], axis=1), wqkv_v[:, cs])
                for jl in range(NQ):
                    put_qkv(b, jl, ct, val[jl * QB:(jl + 1) * QB])
                yield
            return
        for ct in (0, 4, 1, 5, 2, 3):
            cs = slice(ct * 128, (ct + 1) * 128)
            c11, c12, c21, c22 = yield from _strassen(
                lambda i: _dot(lx_s[i * HM:(i + 1) * HM, :], rhs(i, rq_s, HD, quad_q, cs)))
            for jl, c_, val in ((0, ct, c11), (0, ct + HQ // 128, c12), (1, ct, c21), (1, ct + HQ // 128, c22)):
                put_qkv(b, jl, c_, val)
            yield

    def krows(t, j, off, n):
        return k_s[t, pl.ds(al(j * (QB // 2) + off // 2, 8), n // 2), :]

    def scores(j, jl, hq, nt, slot):
        ms = []
        for h in range(4 * hq, 4 * hq + 4):
            qh = qT_s[pl.ds(al(j * HD + h * 8, 8), 8), :]
            if nt == 3:
                w = [jnp.where((lane >= c * SW) & (lane < (c + 1) * SW), qh, np.uint32(0)) for c in range(NSL)]
                lhs, edge = [krows(h, j, -128, 128 + SW)], None
                for c in range(NSL):
                    old = krows(h, j, -256 + c * SW, SW)
                    edge = old if c == 0 else jnp.where(lane >= c * SW, old, edge)
                    if c > 0:
                        lhs.append(jnp.where(lane >= c * SW, krows(h, j, c * SW, SW), old))
                s = _dot(_upk(jnp.concatenate([edge] + lhs, axis=0)), _upk(jnp.concatenate(w, axis=0)))
                r_ = lax.broadcasted_iota(jnp.int32, (SW, QB), 0)
                c_ = lax.broadcasted_iota(jnp.int32, (SW, QB), 1)
                parts = [s[SW:SW + 128]]
                for c in range(NSL):
                    use_old = (c_ >= c * SW) & (c_ < c * SW + r_)
                    parts.append(jnp.where(use_old, s[:SW], s[SW + 128 + c * SW:2 * SW + 128 + c * SW]))
            else:
                w = [qh] + [jnp.zeros((8, QB), U32)] * (NSL - 1)
                s = _dot(_upk(krows(h, j, -128 * (nt - 1), 128 * nt)), _upk(jnp.concatenate(w, axis=0)))
                o = 128 * (nt - 1)
                parts = [s[:o]] * (nt - 1) + [jnp.where(tri, s[o:], NEG)]
            s = jnp.concatenate(parts, axis=0)
            s_s[slot, len(ms), :s.shape[0], :] = s
            ms.append(jnp.max(s, axis=0, keepdims=True))
        return ms

    def finish_steps(pend):
        while True:
            j, jl, hq, nt, slot, ms = pend.pop(0)
            for i in range(4):
                h = 4 * hq + i
                p = jnp.exp2(s_s[slot, i, :128 * min(nt, 2), :] - ms[i])
                l = jnp.sum(p, axis=0, keepdims=True)
                if nt == 3:
                    p = jnp.concatenate([jnp.where(tri, 0.0, p[128:]), p[:128], jnp.where(tri, p[128:], 0.0)], axis=0)
                vh = jnp.concatenate([vT_s[pl.ds(al((j - (nt - 1) + t) * (D // 2) + h * 8, 8), 8), :]
                                      for t in range(nt)], axis=1)
                o = _dot(_upk(vh), p.astype(BF16))
                oT_s[h * DH:(h + 1) * DH, jl * QB:(jl + 1) * QB] = o * (1.0 / l)
                yield

    def score_steps(b, first, pend):
        for u, (jl, hq) in enumerate(UNITS):
            nt = min(jl + 1, 3) if first else 3
            j = b * NQ + jl
            pend.append((j, jl, hq, nt, u % 2, scores(j, jl, hq, nt, u % 2)))
            yield

    def prep_o_steps():
        for c in range(0, HD, 128):
            store_lhs7(lo_s, *(oT_s[f0 + c:f0 + c + 128, t0:t0 + HM].T for t0 in (0, HM) for f0 in (0, HD)),
                       cs=slice(c, c + 128))
            yield

    def proj_steps(b):
        for ct in range(HD // 128):
            cs = slice(ct * 128, (ct + 1) * 128)
            c = yield from _strassen(lambda i: _dot(lo_s[i * HM:(i + 1) * HM, :], rhs(i, ro_s, HD, quad_o, cs)))
            for k in range(4):
                r0, c0 = k // 2 * HM, k % 2 * HD + ct * 128
                h_s[r0:r0 + HM, c0:c0 + 128] = x_v[pl.ds(al(b * BM + r0, HM), HM), c0:c0 + 128].astype(F32) + c[k]
            yield

    def ln2_steps():
        for r in range(0, QM, LN2):
            hn = [_ln(h_s[o + r:o + r + LN2, :], 0.5) for o in range(0, BM, QM)]
            up, dn = (_lhs7(t[:, :HD], t[:, HD:], b_[:, :HD], b_[:, HD:]) for t, b_ in ((hn[0], hn[2]), (hn[1], hn[3])))
            for i in range(7):
                for j, v in enumerate(_lhs7(up[i][:, :128], up[i][:, 128:], dn[i][:, :128], dn[i][:, 128:])):
                    l1_s[((7 * i + j) * QM + r) // 2:((7 * i + j) * QM + r + LN2) // 2, :] = _pk(v.astype(BF16))
            yield

    def prep_gate_up():
        for c0 in range(0, HF, 128):
            for r0 in range(0, 128, 16):
                def blk(n, kr, kc):
                    ref, ro, _ = quad_g[n]
                    return ref[ro + kr + r0:ro + kr + r0 + 16, kc + c0:kc + c0 + 128].astype(F32)
                for i, (n0, sg, n1) in enumerate(RHS_TERMS):
                    q = [blk(n0, kr, kc) if sg == 0 else blk(n0, kr, kc) + blk(n1, kr, kc) if sg > 0
                         else blk(n0, kr, kc) - blk(n1, kr, kc) for kr in (0, 128) for kc in (0, HF)]
                    for j, v in enumerate(_rhs7(*q)):
                        if i not in (1, 4) or j not in (1, 4):
                            rg_s[(7 * i + j) * 128 + r0:(7 * i + j) * 128 + r0 + 16, c0:c0 + 128] = v.astype(BF16)
                yield

    def act(hg, hu):
        return (hg + hg * jnp.tanh(hg)) * hu

    def rhs2(i, j, cs):
        if i in (1, 4) and j in (1, 4):
            ref, ro, _ = quad_g[0 if i == 1 else 3]
            kr, kc = (0, 0) if j == 1 else (128, HF)
            return ref[ro + kr:ro + kr + 128, kc + cs.start:kc + cs.stop]
        return rg_s[(7 * i + j) * 128:(7 * i + j + 1) * 128, cs]

    def gate_up_steps():
        for c in range(NCH):
            cs = slice(c * 128, (c + 1) * 128)
            for i in (4, 2, 0, 6, 3, 1, 5):
                t = yield from _strassen(lambda j: _dot(
                    _upk(l1_s[(7 * i + j) * QM // 2:(7 * i + j + 1) * QM // 2, :]), rhs2(i, j, cs)))
                for k in range(4):
                    if i == 3:
                        part_s[6, k] = act(part_s[0, k] - part_s[4, k] + part_s[6, k] + t[k], part_s[4, k] + part_s[2, k])
                    if i != 5:
                        part_s[i, k] = t[k]
                if i == 5:
                    a_b = [act(part_s[3, k] + part_s[1, k], part_s[0, k] + part_s[2, k] - part_s[1, k] + t[k])
                           for k in range(4)]
                    for k in (0, 2):
                        store_lhs7(l2_s, part_s[6, k], part_s[6, k + 1], a_b[k], a_b[k + 1], cs, k // 2 * QM)
                yield

    T, Bo, Lf, Rt = slice(0, HM), slice(HM, BM), slice(0, HD), slice(HD, D)
    DOWN = [[((T, Lf), 1), ((Bo, Rt), 1)], [((Bo, Lf), 1), ((Bo, Rt), -1)], [((T, Rt), 1), ((Bo, Rt), 1)],
            [((T, Lf), 1), ((Bo, Lf), 1)], [((T, Lf), -1), ((T, Rt), 1)], [((Bo, Rt), 1)], [((T, Lf), 1)]]

    def down_steps(b):
        for i in range(7):
            m = _dot(l2_s[i * HM:(i + 1) * HM, :], rhs(i, rd_s, HF, quad_d, slice(0, HD)))
            for (rs, cs), sg in DOWN[i]:
                seen = [k for k in range(7) if any(q == (rs, cs) for q, _ in DOWN[k])]
                acc = 0.5 * h_s[rs, cs] if i == seen[0] else y_s[rs, cs]
                acc = acc + m if sg > 0 else acc - m
                if i == seen[-1]:
                    out_v[pl.ds(al(b * BM + rs.start, HM), HM), cs] = (2.0 * acc).astype(BF16)
                else:
                    y_s[rs, cs] = acc
            yield

    def start(copies):
        return lambda: [c.start() for c in copies]

    def wait(copies):
        return lambda: [c.wait() for c in copies]

    prep_q = prep_rhs(rq_s, HD, quad_q, [(r, c) for c in range(0, HQ, 128) for r in range(0, HD, 16)])
    prep_w = prep_rhs(ro_s, HD, quad_o, [(r, c) for c in range(0, HD, 128) for r in range(0, HD, 16)])
    prep_f = prep_gate_up()
    prep_d = prep_rhs(rd_s, HF, quad_d, [(r, c) for r in range(0, HF, 16) for c in range(0, HD, 128)])

    def four(g):
        while True:
            for _ in range(4):
                next(g)
            yield

    acts = dict(B=start([x_copies[1]] + sum(w_copies, [])), X=start(x_copies[2:]), Wx0=wait(x_copies[:1]),
                Wx1=wait(x_copies[1:2]), Wx2=wait(x_copies[2:]), Wq=wait(qkv_copies[:1]), Wk=wait(qkv_copies[1:2]), Wv=wait(qkv_copies[2:]), Wo=wait(w_copies[0]),
                Wg=wait(w_copies[1]), Wd=wait(w_copies[2]), C0=start([half_copy(0)]), C1=start([half_copy(1)]))

    def run(order, base):
        gens, pend = {}, {}
        for tok in order.split():
            if tok in acts:
                acts[tok]()
                continue
            kind, b = tok[0], base + int(tok[1:])
            if kind == "c":
                out_copy(b).start()
            elif kind != "z":
                if tok not in gens:
                    first = isinstance(b, int) and b == 0
                    q = pend.setdefault(tok[1:], [])
                    gens[tok] = dict(
                        n=lambda: ln1_steps(b, first), k=lambda: key_steps(b, first), q=lambda: qkv_steps(b, first),
                        s=lambda: score_steps(b, first, q), f=lambda: finish_steps(q), o=prep_o_steps,
                        p=lambda: proj_steps(b), l=ln2_steps, g=gate_up_steps, D=lambda: down_steps(b),
                        t=lambda: prep_q, u=lambda: prep_w, r=lambda: prep_f, d=lambda: four(prep_d))[kind]()
                next(gens[tok])

    head, body, tail = _schedule()
    run(head, 0)

    @pl.loop(1, NB - 1)
    def _(b):
        run(body, b)

    run(tail, NB - 1)
    for c in [out_copy(b) for b in range(NB - 1)] + [half_copy(0), half_copy(1)]:
        c.wait()


@jax.jit
def pallas_sequential_preLN__sliding_block__swiglu_ffn__prompt_kernel(
        A_x, A_wqkv, A_wo, B_x, B_w_gate, B_w_up, B_w_down):
    any_spec = pl.BlockSpec(memory_space=pl.ANY)
    out = pl.pallas_call(
        _kernel,
        out_shape=jax.ShapeDtypeStruct((S, D), BF16),
        in_specs=[any_spec] * 6,
        out_specs=any_spec,
        scratch_shapes=[
            pltpu.VMEM((S, D), BF16), pltpu.VMEM((D, 3 * D), BF16), pltpu.VMEM((D, D), BF16),
            pltpu.VMEM((D, F), BF16), pltpu.VMEM((D, F), BF16), pltpu.VMEM((F, D), BF16), pltpu.VMEM((S, D), BF16),
            pltpu.VMEM((5 * HD // 2, HQ), U32), pltpu.VMEM((5 * HD // 2, HD), U32),
            pltpu.VMEM((49 * 64, HF), U32), pltpu.VMEM((5 * HF // 2, HD), U32),
            pltpu.VMEM((7 * HM // 2, HD), U32), pltpu.VMEM((7 * HM // 2, HD), U32),
            pltpu.VMEM((49 * QM // 2, 128), U32), pltpu.VMEM((7 * HM // 2, HF), U32),
            pltpu.VMEM((D * NQ // 2, QB), U32), pltpu.VMEM((NSL * D // 128, S // 2, 128), U32),
            pltpu.VMEM((S // QB * D // 2, QB), U32), pltpu.VMEM((S // QB * D // 2, QB), U32),
            pltpu.VMEM((D, BM), F32), pltpu.VMEM((2, 4, 256, QB), F32),
            pltpu.VMEM((BM, D), F32), pltpu.VMEM((BM, D), F32), pltpu.VMEM((7, 4, QM, 128), F32),
            pltpu.SemaphoreType.DMA((13,)), pltpu.SemaphoreType.DMA((NB + 1,)),
        ],
        compiler_params=pltpu.CompilerParams(vmem_limit_bytes=100 * 1024 * 1024),
        name="fused_block",
    )(A_x.reshape(S, D), A_wqkv, A_wo, B_w_gate, B_w_up, B_w_down)
    return out.reshape(1, S, D)
```

```python
import numpy as np
import jax
import jax.numpy as jnp
from jax import lax
import jax.experimental.pallas as pl
import jax.experimental.pallas.tpu as pltpu

S, D, H, DH, F = 2048, 512, 32, 16, 1792
QB = 128
F32, BF16, U32 = jnp.float32, jnp.bfloat16, jnp.uint32
QSCALE = float(DH ** -0.5 * np.log2(np.e))
NEG = -1e30
BM = 256
NB, NQ = S // BM, BM // QB
HM, QM, HD, HF, HQ = BM // 2, BM // 4, D // 2, F // 2, 3 * D // 2
NSL, SW = 8, 16
NU = NQ * (H // 4)
NCH = HF // 128
LN1, LN2, KR = 64, 16, 32
UNITS = [(jl, hq) for part in ((0, 1, 4, 5), (2, 3, 6, 7)) for jl in range(NQ) for hq in part]


def _pk(x):
    return pltpu.bitcast(x, U32)


def _upk(x):
    return pltpu.bitcast(x, BF16)


def _dot(a, b):
    return jnp.dot(a, b, preferred_element_type=F32)


def _ln(x, scale=1.0):
    m = jnp.mean(x, axis=-1, keepdims=True)
    c = x - m
    v = jnp.mean(c * c, axis=-1, keepdims=True)
    r = lax.rsqrt(v + 1e-5)
    return c * (r if scale == 1.0 else r * scale)


def _lhs7(a11, a12, a21, a22):
    return [a11 + a22, a21 + a22, a11, a22, a11 + a12, a21 - a11, a12 - a22]


def _rhs5(b11, b12, b21, b22):
    return [b11 + b22, b12 - b22, b21 - b11, b11 + b12, b21 + b22]


def _rhs7(b11, b12, b21, b22):
    return [b11 + b22, b11, b12 - b22, b21 - b11, b22, b11 + b12, b21 + b22]


def _strassen(prod):
    m5 = prod(4)
    yield
    m3 = prod(2)
    c12 = m5 + m3
    yield
    m1 = prod(0)
    c11, c22 = m1 - m5, m1 + m3
    yield
    c11 = c11 + prod(6)
    yield
    m4 = prod(3)
    c11 = c11 + m4
    yield
    m2 = prod(1)
    c21, c22 = m4 + m2, c22 - m2
    yield
    c22 = c22 + prod(5)
    return c11, c12, c21, c22


RHS_SLOT = (0, None, 1, 2, None, 3, 4)
RHS_TERMS = ((0, 1, 3), (0, 0, 0), (1, -1, 3), (2, -1, 0), (3, 0, 0), (0, 1, 1), (2, 1, 3))


def _mix(*streams):
    toks = []
    for s_ in streams:
        t = s_.split()
        if not t:
            continue
        toks += [((i + 0.5) / len(t), len(toks) + i, x) for i, x in enumerate(t)]
    return " ".join(x for _, _, x in sorted(toks)) + " "


def _t(kind, b, n=1):
    return f"{kind}{b} " * n


def _schedule():
    def att(b):
        o = _t("s", b)
        for u in range(NU):
            o += _t("s", b, int(u + 1 < NU)) + _t("f", b, 4) + _t("o", b, int(u + 1 in (NU // 2, NU)))
        return o.split()

    def qk(b):
        return 2 * _mix(_t("q", b, 14), _t("k", b, 2 * NQ * 64 // KR))
    join = " ".join
    ng, nl2, nk = 49 * NCH, QM // LN2, NQ * 64 // KR
    a0, a1 = att(0), att(1)
    head = "Wx0 n0 Wq B " + _t("q", 0, 4) + "Wk q0 " + _mix(_t("q", 0, 3), _t("k", 0, 2 * nk)) + _t("t", 0, 16)
    head += "Wv Wx1 " + _mix(_t("q", 0, 4), _t("k", 0, 2 * nk), _t("t", 0, 8))
    head += _mix(join(a0[:50]), _t("n", 1, HM // LN1) + _t("z", 0, 4) + _t("q", 1, 14), _t("t", 0, 72) + _t("z", 0, 40))
    head += _mix(join(a0[50:]), qk(1)) + "Wo Wg X " + _mix(join(a1[:31]), _t("u", 0, 32) + _t("r", 0, 20))
    head += _mix(join(a1[31:41]), _t("p", 0, 14)) + _mix(join(a1[41:51]), _t("l", 0, nl2))
    head += _mix(join(a1[51:]), _t("g", 0, ng), _t("r", 0, 36) + _t("z", 0, 14)) + "Wd Wx2 " + _t("d", 0, 28)
    body = _mix(_t("D", -1, 3), _t("n", 1, HM // LN1) + "z0") + _t("q", 1, 14) + qk(1) + _t("p", 0, 7)
    body += _mix(_t("p", 0, 7) + _t("z", 0, 7) + _mix(_t("l", 0, nl2), _t("z", 0, 12)), _t("D", -1, 4), join(a1[:16]))
    body += _mix(join(a1[16:]), _t("g", 0, ng)) + _t("c", -1)
    tail = _t("D", -1, 3) + _t("p", 0, 14) + _t("D", -1) + _mix(_t("D", -1, 2), _t("l", 0, nl2)) + _t("D", -1) + _t("c", -1)
    tail += _t("g", 0, ng) + _t("D", 0, 5) + "C2 D0 C1 D0 C0"
    return head, body, tail


def _kernel(x_hbm, wqkv_hbm, wo_hbm, wg_hbm, wu_hbm, wd_hbm, out_hbm,
           x_v, wqkv_v, wo_v, wg_v, wu_v, wd_v, out_v, rq_s, ro_s, rg_s, rd_s,
           lx_s, lo_s, l1_s, l2_s, kt_s, k_s, vT_s, qT_s, oT_s, s_s, h_s, y_s, part_s, in_sem, out_sem):
    rq_s, ro_s, rg_s, rd_s, lx_s, lo_s, l2_s = (
        r.bitcast(BF16) for r in (rq_s, ro_s, rg_s, rd_s, lx_s, lo_s, l2_s))

    def al(i, n):
        return i if isinstance(i, int) else pl.multiple_of(i, n)

    def x_copy(b0, nb, i):
        return pltpu.make_async_copy(x_hbm.at[pl.ds(b0 * BM, nb * BM)], x_v.at[pl.ds(b0 * BM, nb * BM)], in_sem.at[i])

    def out_copy(b):
        r = pl.ds(al(b * BM, BM), BM)
        return pltpu.make_async_copy(out_v.at[r], out_hbm.at[r], out_sem.at[b])

    def last_copy(i):
        r = (pl.ds((NB - 1) * BM + i % 2 * HM, HM), pl.ds(HD * (i // 2), D if i == 1 else HD))
        return pltpu.make_async_copy(out_v.at[r], out_hbm.at[r], out_sem.at[NB - 1 + i])
    x_copies = [x_copy(0, 1, 0), x_copy(1, 1, 1), x_copy(2, NB - 2, 2)]
    sem_ids = iter(range(3, 64))

    def split_copy(src, dst, n):
        rows = src.shape[0] // n
        return [pltpu.make_async_copy(src.at[pl.ds(i * rows, rows)], dst.at[pl.ds(i * rows, rows)],
                                      in_sem.at[next(sem_ids)]) for i in range(n)]
    qkv_copies = [pltpu.make_async_copy(wqkv_hbm.at[:, pl.ds(i * D, D)], wqkv_v.at[:, pl.ds(i * D, D)],
                                        in_sem.at[next(sem_ids)]) for i in range(3)]
    w_copies = [split_copy(wo_hbm, wo_v, 1), split_copy(wg_hbm, wg_v, 2) + split_copy(wu_hbm, wu_v, 2),
                split_copy(wd_hbm, wd_v, 2)]
    x_copies[0].start()
    for c in qkv_copies:
        c.start()

    lane = lax.broadcasted_iota(jnp.int32, (8, QB), 1)
    tri = lax.broadcasted_iota(jnp.int32, (QB, QB), 0) <= lax.broadcasted_iota(jnp.int32, (QB, QB), 1)

    def store_lhs7(dst, a11, a12, a21, a22, cs=slice(None), r0=0):
        for i, a in enumerate(_lhs7(a11, a12, a21, a22)):
            dst[i * HM + r0:i * HM + r0 + a.shape[0], cs] = a.astype(BF16)

    def prep_rhs(dst, kh, quad, tiles):
        for r0, c0 in tiles:
            r = _rhs5(*(ref[ro + r0:ro + r0 + 16, co + c0:co + c0 + 128].astype(F32) for ref, ro, co in quad))
            for i in range(5):
                dst[i * kh + r0:i * kh + r0 + 16, c0:c0 + 128] = r[i].astype(BF16)
            yield

    def rhs(i, pre, kh, quad, cs):
        if RHS_SLOT[i] is None:
            ref, ro, co = quad[0 if i == 1 else 3]
            return ref[ro:ro + kh, co + cs.start:co + cs.stop]
        return pre[RHS_SLOT[i] * kh:(RHS_SLOT[i] + 1) * kh, cs]
    quad_q = ((wqkv_v, 0, 0), (wqkv_v, 0, HQ), (wqkv_v, HD, 0), (wqkv_v, HD, HQ))
    quad_o = ((wo_v, 0, 0), (wo_v, 0, HD), (wo_v, HD, 0), (wo_v, HD, HD))
    quad_g = ((wg_v, 0, 0), (wu_v, 0, 0), (wg_v, HD, 0), (wu_v, HD, 0))
    quad_d = ((wd_v, 0, 0), (wd_v, 0, HD), (wd_v, HF, 0), (wd_v, HF, HD))

    def ln1_steps(b, plain):
        if plain:
            xn = _ln(x_v[b * BM:(b + 1) * BM, :].astype(F32))
            lx_s[0:BM, :], lx_s[BM:2 * BM, :] = xn[:, :HD].astype(BF16), xn[:, HD:].astype(BF16)
            yield
        else:
            for r in range(0, HM, LN1):
                top, bot = (_ln(x_v[pl.ds(al(b * BM + o + r, LN1), LN1), :].astype(F32)) for o in (0, HM))
                store_lhs7(lx_s, top[:, :HD], top[:, HD:], bot[:, :HD], bot[:, HD:], r0=r)
                yield

    def put_qkv(b, jl, ct, val):
        kind, g = divmod(ct, D // 128)
        j = b * NQ + jl
        if kind == 0:
            qT_s[pl.ds(al(j * HD + g * 64, 64), 64), :] = _pk((val * QSCALE).T.astype(BF16))
        elif kind == 2:
            vT_s[pl.ds(al(j * HD + g * 64, 64), 64), :] = _pk(val.T.astype(BF16))
        else:
            kt_s[(g * NQ + jl) * 64:(g * NQ + jl + 1) * 64, :] = _pk(val.astype(BF16))

    def key_steps(b, plain):
        ln_ = lax.broadcasted_iota(jnp.int32, (KR, 128), 1)
        for g in (range(D // 128) if plain else (2, 0, 3, 1)):
            for r in range(0, NQ * 64, KR):
                tiles, w = [kt_s[g * NQ * 64 + r:g * NQ * 64 + r + KR, :]], 64
                while w >= SW:
                    first = (ln_ & w) == 0
                    nxt = []
                    for t in tiles:
                        rot = pltpu.roll(t, w, 1)
                        nxt += [jnp.where(first, t, rot), jnp.where(first, rot, t)]
                    tiles, w = nxt, w // 2
                for i, t in enumerate(tiles):
                    k_s[g * NSL + i, pl.ds(al(b * HM + r, KR), KR), :] = t
                yield

    def qkv_steps(b, plain):
        if plain:
            for ct in range(3 * D // 128):
                cs = slice(ct * 128, (ct + 1) * 128)
                val = _dot(jnp.concatenate([lx_s[0:BM, :], lx_s[BM:2 * BM, :]], axis=1), wqkv_v[:, cs])
                for jl in range(NQ):
                    put_qkv(b, jl, ct, val[jl * QB:(jl + 1) * QB])
                yield
            return
        for ct in (0, 4, 1, 5, 2, 3):
            cs = slice(ct * 128, (ct + 1) * 128)
            c11, c12, c21, c22 = yield from _strassen(
                lambda i: _dot(lx_s[i * HM:(i + 1) * HM, :], rhs(i, rq_s, HD, quad_q, cs)))
            for jl, c_, val in ((0, ct, c11), (0, ct + HQ // 128, c12), (1, ct, c21), (1, ct + HQ // 128, c22)):
                put_qkv(b, jl, c_, val)
            yield

    def krows(t, j, off, n):
        return k_s[t, pl.ds(al(j * (QB // 2) + off // 2, 8), n // 2), :]

    def scores(j, jl, hq, nt, slot):
        ms = []
        for h in range(4 * hq, 4 * hq + 4):
            qh = qT_s[pl.ds(al(j * HD + h * 8, 8), 8), :]
            if nt == 3:
                w = [jnp.where((lane >= c * SW) & (lane < (c + 1) * SW), qh, np.uint32(0)) for c in range(NSL)]
                lhs, edge = [krows(h, j, -128, 128 + SW)], None
                ln_ = lax.broadcasted_iota(jnp.int32, (SW // 2, 128), 1)
                for c in range(NSL):
                    old = krows(h, j, -256 + c * SW, SW)
                    edge = old if c == 0 else jnp.where(ln_ >= c * SW, old, edge)
                    if c > 0:
                        lhs.append(jnp.where(ln_ >= c * SW, krows(h, j, c * SW, SW), old))
                s = _dot(_upk(jnp.concatenate([edge] + lhs, axis=0)), _upk(jnp.concatenate(w, axis=0)))
                r_ = lax.broadcasted_iota(jnp.int32, (SW, QB), 0)
                c_ = lax.broadcasted_iota(jnp.int32, (SW, QB), 1)
                parts = [s[SW:SW + 128]]
                for c in range(NSL):
                    use_old = (c_ >= c * SW) & (c_ < c * SW + r_)
                    parts.append(jnp.where(use_old, s[:SW], s[SW + 128 + c * SW:2 * SW + 128 + c * SW]))
            else:
                w = [qh] + [jnp.zeros((8, QB), U32)] * (NSL - 1)
                s = _dot(_upk(krows(h, j, -128 * (nt - 1), 128 * nt)), _upk(jnp.concatenate(w, axis=0)))
                o = 128 * (nt - 1)
                parts = [s[:o]] * (nt - 1) + [jnp.where(tri, s[o:], NEG)]
            s = jnp.concatenate(parts, axis=0)
            s_s[slot, len(ms), :s.shape[0], :] = s
            ms.append(jnp.max(s, axis=0, keepdims=True))
        return ms

    def finish_steps(pend):
        while True:
            j, jl, hq, nt, slot, ms = pend.pop(0)
            for i in range(4):
                h = 4 * hq + i
                p = jnp.exp2(s_s[slot, i, :128 * min(nt, 2), :] - ms[i])
                l = jnp.sum(p, axis=0, keepdims=True)
                if nt == 3:
                    p = jnp.concatenate([jnp.where(tri, 0.0, p[128:]), p[:128], jnp.where(tri, p[128:], 0.0)], axis=0)
                vh = jnp.concatenate([vT_s[pl.ds(al((j - (nt - 1) + t) * (D // 2) + h * 8, 8), 8), :]
                                      for t in range(nt)], axis=1)
                o = _dot(_upk(vh), p.astype(BF16))
                oT_s[h * DH:(h + 1) * DH, jl * QB:(jl + 1) * QB] = o * (1.0 / l)
                yield

    def score_steps(b, first, pend):
        for u, (jl, hq) in enumerate(UNITS):
            nt = min(jl + 1, 3) if first else 3
            j = b * NQ + jl
            pend.append((j, jl, hq, nt, u % 2, scores(j, jl, hq, nt, u % 2)))
            yield

    def prep_o_steps():
        for c in range(0, HD, 128):
            store_lhs7(lo_s, *(oT_s[f0 + c:f0 + c + 128, t0:t0 + HM].T for t0 in (0, HM) for f0 in (0, HD)),
                       cs=slice(c, c + 128))
            yield

    def proj_steps(b):
        for ct in range(HD // 128):
            cs = slice(ct * 128, (ct + 1) * 128)
            c = yield from _strassen(lambda i: _dot(lo_s[i * HM:(i + 1) * HM, :], rhs(i, ro_s, HD, quad_o, cs)))
            for k in range(4):
                r0, c0 = k // 2 * HM, k % 2 * HD + ct * 128
                h_s[r0:r0 + HM, c0:c0 + 128] = x_v[pl.ds(al(b * BM + r0, HM), HM), c0:c0 + 128].astype(F32) + c[k]
            yield

    def ln2_steps():
        for r in range(0, QM, LN2):
            hn = [_ln(h_s[o + r:o + r + LN2, :], 0.5) for o in range(0, BM, QM)]
            up, dn = (_lhs7(t[:, :HD], t[:, HD:], b_[:, :HD], b_[:, HD:]) for t, b_ in ((hn[0], hn[2]), (hn[1], hn[3])))
            for i in range(7):
                for j, v in enumerate(_lhs7(up[i][:, :128], up[i][:, 128:], dn[i][:, :128], dn[i][:, 128:])):
                    l1_s[((7 * i + j) * QM + r) // 2:((7 * i + j) * QM + r + LN2) // 2, :] = _pk(v.astype(BF16))
            yield

    def prep_gate_up():
        for c0 in range(0, HF, 128):
            for r0 in range(0, 128, 16):
                def blk(n, kr, kc):
                    ref, ro, _ = quad_g[n]
                    return ref[ro + kr + r0:ro + kr + r0 + 16, kc + c0:kc + c0 + 128].astype(F32)
                for i, (n0, sg, n1) in enumerate(RHS_TERMS):
                    q = [blk(n0, kr, kc) if sg == 0 else blk(n0, kr, kc) + blk(n1, kr, kc) if sg > 0
                         else blk(n0, kr, kc) - blk(n1, kr, kc) for kr in (0, 128) for kc in (0, HF)]
                    for j, v in enumerate(_rhs7(*q)):
                        if i not in (1, 4) or j not in (1, 4):
                            rg_s[(7 * i + j) * 128 + r0:(7 * i + j) * 128 + r0 + 16, c0:c0 + 128] = v.astype(BF16)
                yield

    def act(hg, hu):
        return (hg + hg * jnp.tanh(hg)) * hu

    def rhs2(i, j, cs):
        if i in (1, 4) and j in (1, 4):
            ref, ro, _ = quad_g[0 if i == 1 else 3]
            kr, kc = (0, 0) if j == 1 else (128, HF)
            return ref[ro + kr:ro + kr + 128, kc + cs.start:kc + cs.stop]
        return rg_s[(7 * i + j) * 128:(7 * i + j + 1) * 128, cs]

    def gate_up_steps():
        for c in range(NCH):
            cs = slice(c * 128, (c + 1) * 128)
            for i in (4, 2, 0, 6, 3, 1, 5):
                t = yield from _strassen(lambda j: _dot(
                    _upk(l1_s[(7 * i + j) * QM // 2:(7 * i + j + 1) * QM // 2, :]), rhs2(i, j, cs)))
                for k in range(4):
                    if i == 3:
                        part_s[6, k] = act(part_s[0, k] - part_s[4, k] + part_s[6, k] + t[k], part_s[4, k] + part_s[2, k])
                    if i != 5:
                        part_s[i, k] = t[k]
                if i == 5:
                    a_b = [act(part_s[3, k] + part_s[1, k], part_s[0, k] + part_s[2, k] - part_s[1, k] + t[k])
                           for k in range(4)]
                    for k in (0, 2):
                        store_lhs7(l2_s, part_s[6, k], part_s[6, k + 1], a_b[k], a_b[k + 1], cs, k // 2 * QM)
                yield

    T, Bo, Lf, Rt = slice(0, HM), slice(HM, BM), slice(0, HD), slice(HD, D)
    DOWN = [[((T, Lf), 1), ((Bo, Rt), 1)], [((Bo, Lf), 1), ((Bo, Rt), -1)], [((T, Rt), 1), ((Bo, Rt), 1)],
            [((T, Lf), 1), ((Bo, Lf), 1)], [((T, Lf), -1), ((T, Rt), 1)], [((Bo, Rt), 1)], [((T, Lf), 1)]]

    def down_steps(b):
        for i in range(7):
            m = _dot(l2_s[i * HM:(i + 1) * HM, :], rhs(i, rd_s, HF, quad_d, slice(0, HD)))
            for (rs, cs), sg in DOWN[i]:
                seen = [k for k in range(7) if any(q == (rs, cs) for q, _ in DOWN[k])]
                acc = 0.5 * h_s[rs, cs] if i == seen[0] else y_s[rs, cs]
                acc = acc + m if sg > 0 else acc - m
                if i == seen[-1]:
                    out_v[pl.ds(al(b * BM + rs.start, HM), HM), cs] = (2.0 * acc).astype(BF16)
                else:
                    y_s[rs, cs] = acc
            yield

    def start(copies):
        return lambda: [c.start() for c in copies]

    def wait(copies):
        return lambda: [c.wait() for c in copies]

    prep_q = prep_rhs(rq_s, HD, quad_q, [(r, c) for c in range(0, HQ, 128) for r in range(0, HD, 16)])
    prep_w = prep_rhs(ro_s, HD, quad_o, [(r, c) for c in range(0, HD, 128) for r in range(0, HD, 16)])
    prep_f = prep_gate_up()
    prep_d = prep_rhs(rd_s, HF, quad_d, [(r, c) for r in range(0, HF, 16) for c in range(0, HD, 128)])

    def four(g):
        while True:
            for _ in range(4):
                next(g)
            yield

    acts = dict(B=start([x_copies[1]] + sum(w_copies, [])), X=start(x_copies[2:]), Wx0=wait(x_copies[:1]),
                Wx1=wait(x_copies[1:2]), Wx2=wait(x_copies[2:]), Wq=wait(qkv_copies[:1]), Wk=wait(qkv_copies[1:2]), Wv=wait(qkv_copies[2:]), Wo=wait(w_copies[0]),
                Wg=wait(w_copies[1]), Wd=wait(w_copies[2]), C0=start([last_copy(0)]), C1=start([last_copy(1)]), C2=start([last_copy(2)]))

    def run(order, base):
        gens, pend = {}, {}
        for tok in order.split():
            if tok in acts:
                acts[tok]()
                continue
            kind, b = tok[0], base + int(tok[1:])
            if kind == "c":
                out_copy(b).start()
            elif kind != "z":
                if tok not in gens:
                    first = isinstance(b, int) and b == 0
                    q = pend.setdefault(tok[1:], [])
                    gens[tok] = dict(
                        n=lambda: ln1_steps(b, first), k=lambda: key_steps(b, first), q=lambda: qkv_steps(b, first),
                        s=lambda: score_steps(b, first, q), f=lambda: finish_steps(q), o=prep_o_steps,
                        p=lambda: proj_steps(b), l=ln2_steps, g=gate_up_steps, D=lambda: down_steps(b),
                        t=lambda: prep_q, u=lambda: prep_w, r=lambda: prep_f, d=lambda: four(prep_d))[kind]()
                next(gens[tok])

    head, body, tail = _schedule()
    run(head, 0)

    def step(b, carry):
        run(body, b)
        return carry
    lax.fori_loop(1, NB - 1, step, 0)

    run(tail, NB - 1)
    for c in [out_copy(b) for b in range(NB - 1)] + [last_copy(i) for i in range(3)]:
        c.wait()


@jax.jit
def pallas_sequential_preLN__sliding_block__swiglu_ffn__prompt_kernel(
        A_x, A_wqkv, A_wo, B_x, B_w_gate, B_w_up, B_w_down):
    any_spec = pl.BlockSpec(memory_space=pl.ANY)
    out = pl.pallas_call(
        _kernel,
        out_shape=jax.ShapeDtypeStruct((S, D), BF16),
        in_specs=[any_spec] * 6,
        out_specs=any_spec,
        scratch_shapes=[
            pltpu.VMEM((S, D), BF16), pltpu.VMEM((D, 3 * D), BF16), pltpu.VMEM((D, D), BF16),
            pltpu.VMEM((D, F), BF16), pltpu.VMEM((D, F), BF16), pltpu.VMEM((F, D), BF16), pltpu.VMEM((S, D), BF16),
            pltpu.VMEM((5 * HD // 2, HQ), U32), pltpu.VMEM((5 * HD // 2, HD), U32),
            pltpu.VMEM((49 * 64, HF), U32), pltpu.VMEM((5 * HF // 2, HD), U32),
            pltpu.VMEM((7 * HM // 2, HD), U32), pltpu.VMEM((7 * HM // 2, HD), U32),
            pltpu.VMEM((49 * QM // 2, 128), U32), pltpu.VMEM((7 * HM // 2, HF), U32),
            pltpu.VMEM((D * NQ // 2, QB), U32), pltpu.VMEM((NSL * D // 128, S // 2, 128), U32),
            pltpu.VMEM((S // QB * D // 2, QB), U32), pltpu.VMEM((S // QB * D // 2, QB), U32),
            pltpu.VMEM((D, BM), F32), pltpu.VMEM((2, 4, 256, QB), F32),
            pltpu.VMEM((BM, D), F32), pltpu.VMEM((BM, D), F32), pltpu.VMEM((7, 4, QM, 128), F32),
            pltpu.SemaphoreType.DMA((13,)), pltpu.SemaphoreType.DMA((NB + 2,)),
        ],
        compiler_params=pltpu.CompilerParams(vmem_limit_bytes=100 * 1024 * 1024),
        name="fused_block",
    )(A_x.reshape(S, D), A_wqkv, A_wo, B_w_gate, B_w_up, B_w_down)
    return out.reshape(1, S, D)
```
